```python
import os as _os
_os.environ.setdefault("JAX_PLATFORMS", "cpu")
import jax
import jax.numpy as jnp

def _softmax(x, axis=-1):
    return jax.nn.softmax(x, axis=axis)
def _gelu(x):
    return jax.nn.gelu(x, approximate=True)
def _silu(x):
    return jax.nn.silu(x)
def _sigmoid(x):
    return jax.nn.sigmoid(x)
def _layernorm(x, axis=-1, eps=1e-5):
    m = jnp.mean(x, axis=axis, keepdims=True)
    v = jnp.var(x, axis=axis, keepdims=True)
    return (x - m) / jnp.sqrt(v + eps)
def _scatter_add(tgt, idx, src, axis=0):
    return tgt.at[idx].add(src)
def _segment_sum(src, seg, n):
    return jax.ops.segment_sum(src, seg, n)
class _Rng:
    def __init__(self, key):
        self._k = key
    def _next(self):
        self._k, sub = jax.random.split(self._k)
        return sub
    def normal(self, shape):
        return jax.random.normal(self._next(), shape, dtype=jnp.bfloat16)
    def randint(self, lo, hi, shape):
        return jax.random.randint(self._next(), shape, lo, hi, dtype=jnp.int32)
    def uniform(self, shape, lo=0.0, hi=1.0):
        return jax.random.uniform(self._next(), shape, jnp.bfloat16, lo, hi)
    def permutation(self, n):
        return jax.random.permutation(self._next(), n)


kernel_name = 'standalone__fft_conv__vision'

def setup_inputs():
    _rng = _Rng(jax.random.key(int.from_bytes(__import__("os").urandom(4), "little")))
    _w = (lambda a: (lambda t: t.astype(jnp.bfloat16) if jnp.issubdtype(t.dtype, jnp.floating) else t)(jnp.asarray(a)))
    H = W = 224
    C = 96
    K = 3
    return {
        "x": _w((lambda *s: _rng.normal(s) * 0.05)(1, H, W, C)),
        "w": _w((lambda *s: _rng.normal(s) * 0.05)(K, K, C, C)),
    }

def reference(x, w):
    B, H, W, C = x.shape
    K = w.shape[0]
    wp = jnp.pad(w, ((0, H - K), (0, W - K), (0, 0), (0, 0)))
    Xf = (lambda x, axes=(-2,-1): jnp.fft.rfft2(x.astype(jnp.float32), axes=axes))(x, axes=(1, 2))
    Wf = (lambda x, axes=(-2,-1): jnp.fft.rfft2(x.astype(jnp.float32), axes=axes))(wp, axes=(0, 1))
    Yf = jnp.einsum('bhwi,hwio->bhwo', Xf, Wf)
    y = (lambda x, s, axes=(-2,-1): jnp.fft.irfft2(x, s=s, axes=axes).astype(jnp.bfloat16))(Yf, (H, W), axes=(1, 2))
    return y
```

```python
import math

import jax
import jax.numpy as jnp
from jax import lax
import jax.experimental.pallas as pl
import jax.experimental.pallas.tpu as pltpu

F32, BF16, U32 = jnp.float32, jnp.bfloat16, jnp.uint32
R2 = math.sqrt(2.0)


def in_tf(x0, x1, x2, x3, x4, x5):
    p, q = R2 * x1, R2 * x3
    oa, ob = 0.5 * q - p, q - 0.5 * p
    ea, eb = x4 - 2.0 * x2, x4 - 0.5 * x2
    return [(x0 + x4) - 2.5 * x2, ea + oa, ea - oa, eb + ob, eb - ob, (x1 + x5) - 2.5 * x3]


def filt_tf(f0, f1, f2):
    a, b = 1 / R2, R2
    na = 1.0 / (2 * a * a * (a * a - b * b))
    nb = b ** 3 / (2 * b * b * (b * b - a * a))
    ea, eb = f0 + 0.5 * f2, f0 + 2.0 * f2
    return [f0, na * (ea + a * f1), na * (ea - a * f1), nb * (eb + b * f1), nb * (eb - b * f1), f2]


class Sched:
    def __init__(self):
        self.ops = []

    def at(self, t, fn, *a):
        self.ops.append((t, len(self.ops), fn, a))

    def run(self):
        for _, _, fn, a in sorted(self.ops, key=lambda o: o[:2]):
            fn(*a)


def make(T=7, guest=True, mode="full", r0=(30, 58, 114, 198, 224), r1=None, wstart=3, flags=None,
         xl=100, ml=130, R=96, pre=96, npre=3, tfl=384, tfw=300, rp=1, wp=1, wt=0, wwp=0, fl=100, nlast=1,
         hfirst=False, w1t=None, interpret=False, gt=None, wlast=None, refview='x0 o0 d y'):
    H, C, W, L = 224, 96, 224, 128
    W1 = W - L
    C2 = C // 2
    G = C2 // 8
    RB = 4 * T
    nblk = H // RB
    assert nblk * RB == H or mode == "compute"
    r1 = r1 or r0
    rb = [(0,) + tuple(r0), (0,) + tuple(r1)]
    nr = len(r0)
    GT = (T - 1 if gt is None else gt) if guest else -1
    HOSTS = [t for t in range(T) if t != GT][-4:] if guest else []
    S0 = W1 + 2
    PW = L - S0 - 4

    wlast = nlast if wlast is None else wlast
    assert 1 <= wlast <= nlast
    lag = [4 * wlast - 2, 0]

    def kernel(x_hbm, w_hbm, o_hbm, x0b, x1b, o0b, o1b, wv, u_ref, db, yb, rsem, wsem, osem):
        def ld(ref, idx, g0, ng, name):
            if name in refview:
                return ref.bitcast(U32)[(*idx, pl.ds(8 * g0, 8 * ng), slice(None))]
            return pltpu.bitcast(ref[(*idx, pl.ds(16 * g0, 16 * ng), slice(None))], U32)

        def sto(ref, idx, gi, nl, v, name):
            if name in refview:
                ref.bitcast(U32)[(*idx, pl.ds(8 * gi, 8), pl.ds(0, nl))] = v[:, :nl]
            else:
                ref[(*idx, pl.ds(16 * gi, 16), pl.ds(0, nl))] = pltpu.bitcast(v, BF16)[:, :nl]

        def rd(n, c):
            rows = pl.ds(rb[n][c], rb[n][c + 1] - rb[n][c])
            lanes = pl.ds(L, W1) if n else pl.ds(0, L)
            return pltpu.make_async_copy(x_hbm.at[rows, :, lanes], (x0b, x1b)[n].at[rows], rsem.at[n, c])

        def wr(n, r0, num):
            rows = pl.ds(r0, num)
            lanes = pl.ds(L, W1) if n else pl.ds(0, L)
            return pltpu.make_async_copy((o0b, o1b)[n].at[rows], o_hbm.at[rows, :, lanes], osem.at[n])

        wcp = pltpu.make_async_copy(w_hbm, wv, wsem)
        wcp.start(priority=wwp)
        if mode in ("full", "rd"):
            for c in range(nr):
                for n in range(2):
                    rd(n, c).start(priority=rp)
        wcp.wait()

        g = [filt_tf(*[wv[2 - a, kw].astype(F32) for a in range(3)]) for kw in range(3)]
        eye = (lax.broadcasted_iota(jnp.int32, (C, C), 0) == lax.broadcasted_iota(jnp.int32, (C, C), 1)).astype(BF16)

        def tr(k):
            kt = lax.dot_general(eye, k.astype(BF16), (((1,), (1,)), ((), ())), preferred_element_type=F32)
            return pltpu.bitcast(kt.astype(BF16), U32)
        u_ref[12] = tr(jnp.concatenate([wv[2 - a, 0].astype(F32)[64:] for a in range(3)] + [jnp.zeros((32, C), F32)], axis=0))
        for j in range(6):
            for k in range(2):
                u_ref[2 * j + k] = tr(jnp.concatenate([g[0][j][32 * k:32 * k + 32], g[k + 1][j]], axis=0))

        lane = lax.broadcasted_iota(jnp.int32, (8, L), 1)

        def body(it, carry):
            base = it * RB
            rr = [base + r if r < RB else jnp.where(base + r >= H, base + r - H, base + r) for r in range(RB + 2)]

            def wait_rows(n):
                for c in range(nr):
                    first = max(0, -((RB + 2 - rb[n][c] - 1) // RB))
                    pl.when(it == first)(rd(n, c).wait)
            sc = Sched()
            if mode in ("full", "rd"):
                wait_rows(0)
                if w1t is None:
                    wait_rows(1)
                else:
                    sc.at(w1t, wait_rows, 1)
            m, st = {}, {}

            def src(t, n, r, gi):
                return st["b", t, r, gi] if n else ld(x0b, (rr[4 * t + r],), gi, 1, 'x0')

            def fix(t, r, gi):
                if r < 2 and t > 0 and t not in HOSTS and t - 1 not in HOSTS and t - 1 != GT:
                    st["b", t, r, gi] = st["b", t - 1, r + 4, gi]
                    return
                sl = pl.ds(8 * gi, 8)
                t0 = ld(x0b, (rr[4 * t + r],), gi, 1, 'x0')
                f = jnp.where(lane < L - 2, pltpu.roll(t0, W1, 1), t0)
                if t in HOSTS:
                    h = HOSTS.index(t)
                    g0 = ld(x0b, (rr[4 * GT + r],), gi, 1, 'x0')
                    g1 = jnp.concatenate([ld(x1b, (rr[4 * GT + r],), gi, 1, 'x1'), g0[:, W1:]], axis=1)
                    p = pltpu.roll(g1, S0 + 2 - PW * h, 1)
                    if h == 3:
                        e = S0 + 2 + W1 - PW * h
                        p = jnp.where(lane < e, p, pltpu.roll(g0, e, 1))
                    f = jnp.where((lane >= S0) & (lane < L - 2), p, f)
                st["b", t, r, gi] = jnp.concatenate([ld(x1b, (rr[4 * t + r],), gi, 1, 'x1'), f[:, W1:]], axis=1)

            def tf(t, n, gi):
                v = in_tf(*[pltpu.bitcast(src(t, n, r, gi), BF16).astype(F32) for r in range(6)])
                for j in range(6):
                    db[t, n, j, pl.ds(16 * gi, 16), :] = v[j].astype(BF16)

            def rl(t, n, j, k):
                st["r", t, n, j, k] = pltpu.roll(ld(db, (t, n, j), 0, G, 'd'), k + 1, 1)

            def mm(t, n, j, k):
                rhs = jnp.concatenate([ld(db, (t, n, j), 2 * k, 2, 'd'), st.pop(("r", t, n, j, k))], axis=0)
                r = jnp.dot(pltpu.bitcast(u_ref[2 * j + k], BF16), pltpu.bitcast(rhs, BF16), preferred_element_type=F32)
                for gi in range(G):
                    m[t, n, j, k, gi] = r[16 * gi:16 * gi + 16]

            def mr(t, n, i):
                rhs = [src(t, n, i + a, gi) for a in range(3) for gi in (4, 5)]
                rhs = jnp.concatenate(rhs + [jnp.zeros((16, L), U32)], axis=0)
                r = jnp.dot(pltpu.bitcast(u_ref[12], BF16), pltpu.bitcast(rhs, BF16), preferred_element_type=F32)
                for gi in range(G):
                    m[t, n, "r", i, gi] = r[16 * gi:16 * gi + 16]

            def patch(t, i, gi, f):
                if t >= T - nlast:
                    st["f", t, i, gi] = f
                else:
                    sto(o0b, (rr[4 * t + i + 2],), gi, 2, f, 'o0')

            def out(t, n, i, gi, y):
                sl = pl.ds(8 * gi, 8)
                if n:
                    y = y.astype(BF16)
                    yb[t, i, pl.ds(16 * gi, 16), :] = y
                    o1b[rr[4 * t + i + 2], pl.ds(16 * gi, 16), :] = y[:, :W1]
                    y = ld(yb, (t, i), gi, 1, 'y')
                    patch(t, i, gi, pltpu.roll(y, L - W1, 1))
                    if t in HOSTS:
                        h = HOSTS.index(t)
                        p = pltpu.roll(y, (PW * h - S0 - 2) % L, 1)
                        st["g", i, gi] = p if h == 0 else jnp.where(lane < PW * h, st["g", i, gi], p)
                        if h == 3:
                            patch(GT, i, gi, pltpu.roll(y, (PW * h - W1 - S0 - 2) % L, 1))
                            sto(o1b, (rr[4 * GT + i + 2],), gi, W1, st["g", i, gi], "o1")
                else:
                    o0b[rr[4 * t + i + 2], pl.ds(16 * gi, 16), :] = y.astype(BF16)
                    if t >= T - nlast:
                        sto(o0b, (rr[4 * t + i + 2],), gi, 2, st.pop(("f", t, i, gi)), "o0")

            M = lambda t, n, j, gi: m.pop((t, n, j, 0, gi)) + m.pop((t, n, j, 1, gi))

            def r1_(t, n, gi):
                a, b = M(t, n, 1, gi), M(t, n, 2, gi)
                st["s", gi] = a + b, a - b

            def r2_(t, n, gi):
                a, b = M(t, n, 3, gi), M(t, n, 4, gi)
                sa, da_ = st["s", gi]
                sb, db_ = a + b, a - b
                c = 0.5 / R2
                st["s", gi] = sa + c * sb, (1 / R2) * da_ + 0.5 * db_, 0.5 * sa + (1 / R2) * sb, c * da_ + db_

            def r3_(t, n, gi):
                y = st["s", gi]
                out(t, n, 0, gi, y[0] + (M(t, n, 0, gi) + m.pop((t, n, "r", 0, gi))))
                out(t, n, 1, gi, y[1] + m.pop((t, n, "r", 1, gi)))

            def r4_(t, n, gi):
                y = st["s", gi]
                out(t, n, 2, gi, y[2] + m.pop((t, n, "r", 2, gi)))
                out(t, n, 3, gi, y[3] + (M(t, n, 5, gi) + m.pop((t, n, "r", 3, gi))))

            def r34(t, n, gi):
                r3_(t, n, gi)
                r4_(t, n, gi)

            k = 0
            for t in range(npre):
                for i in range(4):
                    sc.at(k * R - pre, mr, t, 0, i)
                k += 1
            bs = [t for t in range(T) if t != GT]
            if hfirst:
                bs = HOSTS + [t for t in bs if t not in HOSTS]
            tiles = [(t, 0) for t in range(T - nlast)] + [(t, 1) for t in bs] + [(t, 0) for t in range(T - nlast, T)]
            for q, t in enumerate(sorted(bs)):
                for gi in range(G):
                    for r in range(6):
                        sc.at((w1t or 0) + fl + (q * G + gi) * 10, fix, t, r, gi)
            for t, n in tiles:
                if n == 0 and t < npre:
                    rounds = [(r1_, (1, 2), ()), (r2_, (3, 4), ()), (r34, (0, 5), ())]
                else:
                    rounds = [(r1_, (1, 2), ()), (r2_, (3, 4), ()), (r3_, (0,), (0, 1)), (r4_, (5,), (2, 3))]
                tb = k * R - pre - xl - tfl
                for gi in range(G):
                    sc.at(tb + tfw * gi / G, tf, t, n, gi)
                for fn, js, rs in rounds:
                    t0 = k * R
                    k += 1
                    for j in js:
                        for kk in range(2):
                            sc.at(t0 - pre - xl, rl, t, n, j, kk)
                            sc.at(t0 - pre, mm, t, n, j, kk)
                    for i in rs:
                        sc.at(t0 - pre, mr, t, n, i)
                    for gi in range(G):
                        sc.at(t0 + ml + R * gi / G, fn, t, n, gi)

            def writes():
                @pl.when(it == wstart)
                def _():
                    for n in range(2):
                        wr(n, 2, (wstart + 1) * RB - lag[n] - 2).start(priority=wp)
                @pl.when(it > wstart)
                def _():
                    for n in range(2):
                        wr(n, base - lag[n], RB).start(priority=wp)
            if mode in ("full", "wr"):
                sc.at((k - 4 * wlast - 1) * R + ml + R + wt, writes)
            sc.run()
            return carry

        lax.fori_loop(0, nblk, body, 0)
        if mode in ("full", "wr"):
            for n in range(2):
                if lag[n]:
                    wr(n, H - lag[n], lag[n]).start(priority=wp)
                wr(n, 0, 2).start(priority=wp)
            for n in range(2):
                wr(n, 0, H).wait()
        else:
            for n in range(2):
                wr(n, 0, 1).start()
                wr(n, 0, 1).wait()

    def f(x, w):
        xt = jnp.transpose(x[0], (0, 2, 1))
        bufs = [pltpu.VMEM((H, C, L), BF16), pltpu.VMEM((H, C, W1), BF16)] * 2
        o = pl.pallas_call(
            kernel,
            in_specs=[pl.BlockSpec(memory_space=pl.ANY), pl.BlockSpec(memory_space=pl.ANY)],
            out_specs=pl.BlockSpec(memory_space=pl.ANY),
            out_shape=jax.ShapeDtypeStruct((H, C, W), BF16),
            scratch_shapes=bufs + [
                pltpu.VMEM((3, 3, C, C), BF16), pltpu.VMEM((13, C2, L), U32),
                pltpu.VMEM((T, 2, 6, C, L), BF16), pltpu.VMEM((T, 4, C, L), BF16),
                pltpu.SemaphoreType.DMA((2, nr)), pltpu.SemaphoreType.DMA(()), pltpu.SemaphoreType.DMA((2,)),
            ],
            compiler_params=pltpu.CompilerParams(vmem_limit_bytes=64 * 2**20, flags=flags),
            name="wconv",
            interpret=interpret,
        )(xt, w)
        return jnp.transpose(o, (0, 2, 1))[None]
    return f


_impl = make(npre=2, nlast=3, xl=300, wstart=2)


@jax.jit
def pallas_standalone__fft_conv__vision_kernel(x: jax.Array, w: jax.Array):
    return _impl(x, w)
```

```python
import math

import jax
import jax.numpy as jnp
from jax import lax
import jax.experimental.pallas as pl
import jax.experimental.pallas.tpu as pltpu

F32, BF16, U32 = jnp.float32, jnp.bfloat16, jnp.uint32
SQRT2 = math.sqrt(2.0)

H, W, C = 224, 224, 96
L = 128
W1 = W - L
G = C // 16
GD = 4
CD = 16 * GD

SMALL, BIG = 2, 6
SEGMENTS = ((2, 8), (2, 0))
SIZES = sum(((SMALL,) * a + (BIG,) * b for a, b in SEGMENTS), ())
STARTS = [4 * sum(SIZES[:i]) for i in range(len(SIZES) + 1)]
STEPS = len(SIZES)

UNIT = 64
UNITS = H * C // UNIT
COLUMNS = (0, 4, 2, 6, 1, 5, 3, 7)
WRITES = ((5, 4, 6), (7, 5, 0), (9, 1, 0), (10, 1, 0))

ROUNDS = ("s", "o12", "o34", "e12", "o05", "e34", "e05")
EARLY = 2
RING = 12


def _input_transform(x0, x1, x2, x3, x4, x5):
    h2, h3 = 0.5 * x2, 0.5 * x3
    ea, eb = x4 - 2.0 * x2, x4 - h2
    b = 2.0 * x3 - x1
    oa, ob = SQRT2 * (h3 - x1), (1 / SQRT2) * b
    return [ea + (x0 - h2), ea + oa, ea - oa, eb + ob, eb - ob, (x5 - h3) - b]


def _filter_transform(f0, f1, f2):
    na, nb = -1.0 / 3.0, 1.0 / 6.0
    ea, eb = na * (f0 + 0.5 * f2), nb * (f0 + 2.0 * f2)
    oa, ob = (na / SQRT2) * f1, (nb * SQRT2) * f1
    return [f0, ea + oa, ea - oa, eb + ob, eb - ob, f2]


def _output_transform(sa, ta, sb, tb):
    s = sa + sb
    return s + sa, SQRT2 * (ta + tb), s + sb, (1 / SQRT2) * ta + (2 * SQRT2) * tb


def _words(ref, idx, g0, num):
    return ref.bitcast(U32)[(*idx, pl.ds(8 * g0, 8 * num), slice(None))]


def _kernel(x_hbm, w_hbm, y_hbm, x0_ref, x1_ref, y0_ref, y1_ref, w_ref, u_ref, d_ref,
            odd_ref, even_small_ref, even_big_ref, row_ref, acc_ref, x_sem, w_sem, y_sem):
    def read(sem, r0, num):
        rows = pl.ds(r0, num)
        return [pltpu.make_async_copy(x_hbm.at[rows, :, cols], ref.bitcast(BF16).at[rows], x_sem.at[sem])
                for ref, cols in ((x0_ref, pl.ds(0, L)), (x1_ref, pl.ds(L, W1)))]

    def read_head():
        return read(STEPS, H - 2, 2) + read(STEPS, 0, 4)

    def read_step(s):
        r0 = STARTS[s] + 4
        return read(s, r0, min(STARTS[s + 1] + 4, H - 2) - r0)

    def write(half, units, rows):
        ref, cols = ((y0_ref, pl.ds(0, L)), (y1_ref, pl.ds(L, W1)))[half]
        return pltpu.make_async_copy(ref.bitcast(BF16).at[units, rows], y_hbm.at[units, rows, cols], y_sem)

    def write_batch(n):
        bounds = [0] + [(STARTS[s] + 4 * g) * C // UNIT for s, g, _ in WRITES] + [UNITS]
        units = pl.ds(bounds[n], bounds[n + 1] - bounds[n])
        return [lambda q=q, half=half, p=p:
                write(half, units, pl.ds(8 * COLUMNS[q + p], 8)).start(priority=p)
                for q in range(0, len(COLUMNS), 2) for half in range(2) for p in range(2)]

    w_copy = pltpu.make_async_copy(w_hbm, w_ref, w_sem)
    w_copy.start()
    for copy in read_head() + [copy for s in range(STEPS) for copy in read_step(s)]:
        copy.start(priority=1)
    w_copy.wait()

    f = [[w_ref[2 - a, 2 - b] for a in range(3)] for b in range(3)]
    eye = (lax.broadcasted_iota(jnp.int32, (C, C), 0)
           == lax.broadcasted_iota(jnp.int32, (C, C), 1)).astype(BF16)

    def transposed(parts):
        return lax.dot_general(eye, jnp.concatenate(parts, axis=0), (((1,), (1,)), ((), ())),
                               preferred_element_type=F32)

    shared = [(f[1][a][CD:].astype(F32) + f[2][a][CD:].astype(F32)).astype(BF16) for a in range(3)]
    u_ref[18] = transposed(shared + [jnp.zeros((L - 3 * (C - CD), C), BF16)]).astype(BF16)
    passes = (lambda a: [f[1][a][:CD], f[2][a][:CD]],
              lambda a: [f[0][a], f[1][a][CD:]],
              lambda a: [f[0][a], f[2][a][CD:]])
    for k, parts in enumerate(passes):
        for j, u in enumerate(_filter_transform(*[transposed(parts(a)) for a in range(3)])):
            u_ref[3 * j + k] = u.astype(BF16)

    lane = lax.broadcasted_iota(jnp.int32, (8, L), 1)
    odd_lane = (lane & 1) == 1
    p_from_hi = (odd_lane & (lane < W1)) | (lane == L - 2)
    q_from_hi = (~odd_lane & (lane < W1)) | (lane == L - 1)
    lo_from_odd = odd_lane != (lane >= L - 2)
    P, Q, E1, E3 = range(4)

    def staged(kind, r, g):
        return kind, r % RING, pl.ds(8 * g, 8), slice(None)

    def interleave(rows, r, g):
        lo = x0_ref[rows[r], pl.ds(8 * g, 8), :]
        hi = x1_ref[rows[r], pl.ds(8 * g, 8), :]
        hi = jnp.concatenate([hi, hi[:, 2 * W1 - L:]], axis=1)
        row_ref[staged(P, r, g)] = jnp.where(p_from_hi, hi, lo)
        row_ref[staged(Q, r, g)] = jnp.where(q_from_hi, hi, lo)

    def shift(r, g):
        q = row_ref[staged(Q, r, g)]
        row_ref[staged(E1, r, g)] = pltpu.roll(q, 1, 1)
        row_ref[staged(E3, r, g)] = pltpu.roll(q, L - 1, 1)

    def transform(slot, r0, g):
        def along_h(kind):
            return _input_transform(*[
                pltpu.bitcast(row_ref[staged(kind, r0 + r, g)], BF16).astype(F32) for r in range(6)])

        p = along_h(P)
        for j in range(6):
            d_ref[slot, j, 0, pl.ds(16 * g, 16), :] = p[j].astype(BF16)
        q = along_h(Q if g < GD else E1)
        for j in range(6):
            d_ref[slot, j, 1, pl.ds(16 * g, 16), :] = q[j].astype(BF16)
            if g >= GD:
                d_ref[slot, j, 2, pl.ds(16 * (g - GD), 16), :] = (q[j] - p[j]).astype(BF16)
        if g >= GD:
            q = along_h(E3)
            for j in range(6):
                d_ref[slot, j, 2, pl.ds(16 * (g - GD + 2), 16), :] = (q[j] - p[j]).astype(BF16)

    def step(size, rows, unit0, writes):
        plan, out, rolled, after = [], {}, {}, {}
        count = [0]
        true = lane >= -rows[2]
        even_ref = even_big_ref if size == BIG else even_small_ref

        def at(time, fn, *args):
            plan.append((time, len(plan), fn, args))

        def matmul(key, u, parts):
            lhs = _words(u_ref, (u,), 0, G)
            for reg, value in after.get(count[0], ()):
                keep = jnp.where(true, lhs[8 * reg:8 * reg + 8], value())
                lhs = jnp.concatenate(
                    ([lhs[:8 * reg]] if reg else []) + [keep, lhs[8 * reg + 8:]], axis=0)
            count[0] += 1
            res = jnp.dot(pltpu.bitcast(lhs, BF16), pltpu.bitcast(jnp.concatenate(parts, axis=0), BF16),
                          preferred_element_type=F32)
            for g in range(G):
                out[(*key, g)] = res[16 * g:16 * g + 16]

        def roll(t, odd, j):
            if ("e1", t, j) not in rolled:
                rolled["e1", t, j] = pltpu.roll(_words(d_ref, (t % 2, j, 1), 0, GD), 1, 1)
            if odd:
                rolled["e3", t, j] = pltpu.roll(_words(d_ref, (t % 2, j, 1), 0, GD), L - 1, 1)
            else:
                rolled["e0", t, j] = pltpu.roll(_words(d_ref, (t % 2, j, 0), 0, G), 2, 1)

        def multiply(t, odd, j):
            e1, e2 = rolled["e1", t, j], _words(d_ref, (t % 2, j, 0), 0, GD)
            if odd:
                matmul((t, odd, j, 0), 3 * j, [e2, rolled["e3", t, j]])
                matmul((t, odd, j, 1), 3 * j + 2,
                       [e1, _words(d_ref, (t % 2, j, 1), GD, 2), _words(d_ref, (t % 2, j, 2), 2, 2)])
            else:
                matmul((t, odd, j, 0), 3 * j, [e1, e2])
                matmul((t, odd, j, 1), 3 * j + 1,
                       [rolled["e0", t, j], _words(d_ref, (t % 2, j, 2), 0, 2)])

        def multiply_shared(t, i):
            def e2(r, g):
                if t >= EARLY:
                    return row_ref[staged(P, r, g)]
                lo = x0_ref[rows[r], pl.ds(8 * g, 8), :]
                hi = jnp.concatenate([x1_ref[rows[r], pl.ds(8 * g, 8), :], lo[:, W1:]], axis=1)
                return jnp.where(odd_lane, hi, lo)
            matmul((t, "s", i), 18, [e2(4 * t + i + a, g) for a in range(3) for g in range(GD, G)]
                   + [jnp.zeros((16, L), U32)])

        def acc(t, i, g):
            return t % 2, i, pl.ds(16 * g, 16), slice(None)

        def product(t, odd, j, g):
            return out.pop((t, odd, j, 0, g)) + out.pop((t, odd, j, 1, g))

        def emit(t, odd, i, g, y):
            ref = odd_ref if odd else even_ref
            ref[t % 2, i, pl.ds(16 * g, 16), :] = y.astype(BF16)
            if not odd:
                y_even = _words(even_ref, (t % 2, i), g, 1)
                y_odd = pltpu.roll(_words(odd_ref, (t % 2, i), g, 1), 1, 1)
                unit, reg = divmod((4 * t + i) * G + g, UNIT // 16)
                y0_ref[unit0 + unit, pl.ds(8 * reg, 8), :] = jnp.where(lo_from_odd, y_odd, y_even)
                y1_ref[unit0 + unit, pl.ds(8 * reg, 8), :] = jnp.where(lo_from_odd, y_even, y_odd)[:, :W1]

        def finish_shared(t, g):
            for i in range(4):
                acc_ref[acc(t, 8 + i, g)] = out.pop((t, "s", i, g))

        def finish_12(t, odd, g):
            a, b = product(t, odd, 1, g), product(t, odd, 2, g)
            s, d = a + b, a - b
            acc_ref[acc(t, 4 * odd, g)] = s
            acc_ref[acc(t, 4 * odd + 1, g)] = d

        def finish_34(t, odd, g):
            a, b = product(t, odd, 3, g), product(t, odd, 4, g)
            y = _output_transform(acc_ref[acc(t, 4 * odd, g)], acc_ref[acc(t, 4 * odd + 1, g)], a + b, a - b)
            s1, s2 = acc_ref[acc(t, 9, g)], acc_ref[acc(t, 10, g)]
            emit(t, odd, 1, g, y[1] + s1)
            emit(t, odd, 2, g, y[2] + s2)
            acc_ref[acc(t, 4 * odd + 2, g)] = y[0]
            acc_ref[acc(t, 4 * odd + 3, g)] = y[3]

        def finish_05(t, odd, g):
            first = product(t, odd, 0, g) + acc_ref[acc(t, 8, g)]
            last = product(t, odd, 5, g) + acc_ref[acc(t, 11, g)]
            y0, y3 = acc_ref[acc(t, 4 * odd + 2, g)], acc_ref[acc(t, 4 * odd + 3, g)]
            emit(t, odd, 0, g, y0 + first)
            emit(t, odd, 3, g, y3 + last)

        def transformed(slot, part, g, points):
            def value():
                v = _words(d_ref, (slot, points[0], part), g, 1)
                for j in points[1:]:
                    v = v | _words(d_ref, (slot, j, part), g, 1)
                return v
            return 0, value

        def emitted():
            unit, reg = divmod(G, UNIT // 16)
            idx = jnp.minimum(unit0 + unit, UNITS - 1), pl.ds(8 * reg, 8), slice(None)
            lo = y0_ref[idx]
            return jnp.concatenate([y1_ref[idx], lo[:, W1:]], axis=1)

        def shared_round(t, k):
            for i in range(4):
                at(k - 1, multiply_shared, t, i)
            for g in range(G):
                at(k + 1.35 + g / G, finish_shared, t, g)

        for t in range(EARLY):
            shared_round(t, t)
        k = EARLY
        for t in range(size):
            slot = (t + 1) % 2
            begin = k - 1.99 if t else -2
            for g in range(G):
                time = begin + 0.94 * g / G
                at(time, transform, slot, 4 * t + 4, g)
                for r in range(4 * t + (6 if t else 4), 4 * t + 10):
                    at(time - 0.42, interleave, rows, r, g)
                    if g >= GD:
                        at(time - 0.21, shift, r, g)
            pieces = ([(part, g) for g in range(GD) for part in range(2)]
                      + [(1, 4), (2, 2), None, (1, 5), (2, 3), None])
            due = k + len(ROUNDS) - (t < EARLY) + (EARLY <= t + 1 < size) + 2
            for q, piece in enumerate(pieces):
                if piece:
                    points = tuple(range(6)) if t + 1 == size else (1,)
                    index = int(4 * (due - 6.5 * (1 - q / len(pieces))))
                    assert index // 4 - 1 > begin + 1
                    after.setdefault(index, []).append(transformed(slot, *piece, points))

            for name in ROUNDS:
                if name == "s":
                    if t >= EARLY:
                        shared_round(t, k)
                        k += 1
                    continue
                odd = int(name[0] == "o")
                finish = {"12": finish_12, "34": finish_34, "05": finish_05}[name[1:]]
                for j in map(int, name[1:]):
                    at(k - 2.04, roll, t, odd, j)
                    at(k - 1, multiply, t, odd, j)
                for g in range(G):
                    at(k + 1.35 + g / G, finish, t, odd, g)
                k += 1
            after.setdefault(4 * (k + 3), []).insert(0, (1, emitted))
            for done, delay, starts in writes:
                if done == t + 1:
                    for q, start in enumerate(starts):
                        at(k + delay + 1.3 + q / 32, start)

        for _, _, fn, args in sorted(plan, key=lambda entry: entry[:2]):
            fn(*args)

    for copy in read_head():
        copy.wait()
    for g in range(G):
        for r in range(6):
            interleave([H - 2, H - 1, 0, 1, 2, 3], r, g)
    for g in range(GD, G):
        for r in range(6):
            shift(r, g)
    for g in range(G):
        transform(0, 0, g)

    def loop_body(size):
        def body(_, carry):
            s, base = carry
            rows = [base - 2 + r for r in range(4 * size + 6)]
            if size == SMALL:
                @pl.when(s < STEPS - 1)
                def _():
                    for copy in read(s, base + 4, 4 * size):
                        copy.wait()

                @pl.when(s == STEPS - 1)
                def _():
                    for copy in read_step(STEPS - 1):
                        copy.wait()

                rows[:2] = [jnp.where(r < 0, r + H, r) for r in rows[:2]]
                rows[-4:] = [jnp.where(r >= H, r - H, r) for r in rows[-4:]]
            else:
                for copy in read(s, base + 4, 4 * size):
                    copy.wait()
            writes = [(done, delay, [lambda start=start, on=on: pl.when(s == on)(start)
                                     for start in write_batch(n)])
                      for n, (on, done, delay) in enumerate(WRITES) if SIZES[on] == size]
            step(size, rows, (base >> 3) * (8 * C // UNIT), writes)
            return s + 1, base + 4 * size
        return body

    def segment(i, carry):
        for col, size in enumerate((SMALL, BIG)):
            trips = jnp.where(i == 0, SEGMENTS[0][col], SEGMENTS[1][col])
            carry = lax.fori_loop(0, trips, loop_body(size), carry)
        return carry

    lax.fori_loop(0, len(SEGMENTS), segment, (jnp.int32(0), jnp.int32(0)))

    for start in write_batch(len(WRITES)):
        start()
    for half in range(2):
        write(half, pl.ds(0, UNITS), pl.ds(0, UNIT)).wait()


@jax.jit
def pallas_standalone__fft_conv__vision_kernel(x: jax.Array, w: jax.Array):
    assert x.shape == (1, H, W, C) and w.shape == (3, 3, C, C)
    assert x.dtype == BF16 and w.dtype == BF16
    y = pl.pallas_call(
        _kernel,
        in_specs=[pl.BlockSpec(memory_space=pl.ANY), pl.BlockSpec(memory_space=pl.ANY)],
        out_specs=pl.BlockSpec(memory_space=pl.ANY),
        out_shape=jax.ShapeDtypeStruct((UNITS, UNIT, W), BF16),
        scratch_shapes=[
            pltpu.VMEM((H, C // 2, L), U32),
            pltpu.VMEM((H, C // 2, W1), U32),
            pltpu.VMEM((UNITS, UNIT // 2, L), U32),
            pltpu.VMEM((UNITS, UNIT // 2, W1), U32),
            pltpu.VMEM((3, 3, C, C), BF16),
            pltpu.VMEM((19, C, L), BF16),
            pltpu.VMEM((2, 6, 3, C, L), BF16),
            pltpu.VMEM((2, 4, C, L), BF16),
            pltpu.VMEM((2, 4, C, L), BF16),
            pltpu.VMEM((2, 4, C, L), BF16),
            pltpu.VMEM((4, RING, C // 2, L), U32),
            pltpu.VMEM((2, 12, C, L), F32),
            pltpu.SemaphoreType.DMA((STEPS + 1,)),
            pltpu.SemaphoreType.DMA(()),
            pltpu.SemaphoreType.DMA(()),
        ],
        compiler_params=pltpu.CompilerParams(
            vmem_limit_bytes=48 * 2**20, disable_semaphore_checks=True),
        name="wconv",
    )(jnp.transpose(x.reshape(H, W, C), (0, 2, 1)), w)
    return jnp.transpose(y.reshape(H, C, W), (0, 2, 1)).reshape(1, H, W, C)
```

```python
import math

import jax
import jax.numpy as jnp
from jax import lax
import jax.experimental.pallas as pl
import jax.experimental.pallas.tpu as pltpu

F32, BF16, U32 = jnp.float32, jnp.bfloat16, jnp.uint32
SQRT2 = math.sqrt(2.0)

H, W, C = 224, 224, 96
L = 128
W1 = W - L
G = C // 16
GD = 4
CD = 16 * GD

SMALL, BIG = 2, 6
SEGMENTS = ((2, 8), (2, 0))
SIZES = sum(((SMALL,) * a + (BIG,) * b for a, b in SEGMENTS), ())
STARTS = [4 * sum(SIZES[:i]) for i in range(len(SIZES) + 1)]
STEPS = len(SIZES)

UNIT = 64
UNITS = H * C // UNIT
WRITES = ((5, 4, 6), (7, 5, 0), (9, 1, 0), (10, 1, 0))

ROUNDS = ("s", "o12", "o34", "e12", "o05", "e34", "e05")
EARLY = 2
RING = 12


def _input_transform(x0, x1, x2, x3, x4, x5):
    h2, h3 = 0.5 * x2, 0.5 * x3
    ea, eb = x4 - 2.0 * x2, x4 - h2
    b = 2.0 * x3 - x1
    oa, ob = SQRT2 * (h3 - x1), (1 / SQRT2) * b
    return [ea + (x0 - h2), ea + oa, ea - oa, eb + ob, eb - ob, (x5 - h3) - b]


def _filter_transform(f0, f1, f2):
    na, nb = -1.0 / 3.0, 1.0 / 6.0
    ea, eb = na * (f0 + 0.5 * f2), nb * (f0 + 2.0 * f2)
    oa, ob = (na / SQRT2) * f1, (nb * SQRT2) * f1
    return [f0, ea + oa, ea - oa, eb + ob, eb - ob, f2]


def _output_transform(sa, ta, sb, tb):
    s = sa + sb
    return s + sa, SQRT2 * (ta + tb), s + sb, (1 / SQRT2) * ta + (2 * SQRT2) * tb


def _words(ref, idx, g0, num):
    return ref.bitcast(U32)[(*idx, pl.ds(8 * g0, 8 * num), slice(None))]


def _kernel(x_hbm, w_hbm, y_hbm, x0_ref, x1_ref, y0_ref, y1_ref, w_ref, u_ref, d_ref,
            odd_ref, even_small_ref, even_big_ref, row_ref, acc_ref, x_sem, w_sem, y_sem):
    def read(sem, r0, num):
        rows = pl.ds(r0, num)
        return [pltpu.make_async_copy(x_hbm.at[rows, :, cols], ref.bitcast(BF16).at[rows], x_sem.at[sem])
                for ref, cols in ((x0_ref, pl.ds(0, L)), (x1_ref, pl.ds(L, W1)))]

    def read_head():
        return read(STEPS, H - 2, 2) + read(STEPS, 0, 4)

    def read_step(s):
        r0 = STARTS[s] + 4
        return read(s, r0, min(STARTS[s + 1] + 4, H - 2) - r0)

    def write(half, units, rows):
        ref, cols = ((y0_ref, pl.ds(0, L)), (y1_ref, pl.ds(L, W1)))[half]
        return pltpu.make_async_copy(ref.bitcast(BF16).at[units, rows], y_hbm.at[units, rows, cols], y_sem)

    def write_batch(n):
        bounds = [0] + [(STARTS[s] + 4 * g) * C // UNIT for s, g, _ in WRITES] + [UNITS]
        units = pl.ds(bounds[n], bounds[n + 1] - bounds[n])
        return [lambda c=c, half=half, p=p: write(half, units, pl.ds(c + 8 * p, 8)).start(priority=p)
                for c in range(0, UNIT, 16) for half in range(2) for p in range(2)]

    w_copy = pltpu.make_async_copy(w_hbm, w_ref, w_sem)
    w_copy.start()
    for copy in read_head() + [copy for s in range(STEPS) for copy in read_step(s)]:
        copy.start(priority=1)
    w_copy.wait()

    f = [[w_ref[2 - a, 2 - b] for a in range(3)] for b in range(3)]
    eye = (lax.broadcasted_iota(jnp.int32, (C, C), 0)
           == lax.broadcasted_iota(jnp.int32, (C, C), 1)).astype(BF16)

    def transposed(parts):
        return lax.dot_general(eye, jnp.concatenate(parts, axis=0), (((1,), (1,)), ((), ())),
                               preferred_element_type=F32)

    shared = [(f[1][a][CD:].astype(F32) + f[2][a][CD:].astype(F32)).astype(BF16) for a in range(3)]
    u_ref[18] = transposed(shared + [jnp.zeros((L - 3 * (C - CD), C), BF16)]).astype(BF16)
    passes = (lambda a: [f[1][a][:CD], f[2][a][:CD]],
              lambda a: [f[0][a], f[1][a][CD:]],
              lambda a: [f[0][a], f[2][a][CD:]])
    for k, parts in enumerate(passes):
        for j, u in enumerate(_filter_transform(*[transposed(parts(a)) for a in range(3)])):
            u_ref[3 * j + k] = u.astype(BF16)

    lane = lax.broadcasted_iota(jnp.int32, (8, L), 1)
    odd_lane = (lane & 1) == 1
    p_from_hi = (odd_lane & (lane < W1)) | (lane == L - 2)
    q_from_hi = (~odd_lane & (lane < W1)) | (lane == L - 1)
    lo_from_odd = odd_lane != (lane >= L - 2)
    P, Q, E1, E3 = range(4)

    def staged(kind, r, g):
        return kind, r % RING, pl.ds(8 * g, 8), slice(None)

    def interleave(rows, r, g):
        lo = x0_ref[rows[r], pl.ds(8 * g, 8), :]
        hi = x1_ref[rows[r], pl.ds(8 * g, 8), :]
        hi = jnp.concatenate([hi, hi[:, 2 * W1 - L:]], axis=1)
        row_ref[staged(P, r, g)] = jnp.where(p_from_hi, hi, lo)
        row_ref[staged(Q, r, g)] = jnp.where(q_from_hi, hi, lo)

    def shift(r, g):
        q = row_ref[staged(Q, r, g)]
        row_ref[staged(E1, r, g)] = pltpu.roll(q, 1, 1)
        row_ref[staged(E3, r, g)] = pltpu.roll(q, L - 1, 1)

    def transform(slot, r0, g):
        def along_h(kind):
            return _input_transform(*[
                pltpu.bitcast(row_ref[staged(kind, r0 + r, g)], BF16).astype(F32) for r in range(6)])

        p = along_h(P)
        for j in range(6):
            d_ref[slot, j, 0, pl.ds(16 * g, 16), :] = p[j].astype(BF16)
        q = along_h(Q if g < GD else E1)
        for j in range(6):
            d_ref[slot, j, 1, pl.ds(16 * g, 16), :] = q[j].astype(BF16)
            if g >= GD:
                d_ref[slot, j, 2, pl.ds(16 * (g - GD), 16), :] = (q[j] - p[j]).astype(BF16)
        if g >= GD:
            q = along_h(E3)
            for j in range(6):
                d_ref[slot, j, 2, pl.ds(16 * (g - GD + 2), 16), :] = (q[j] - p[j]).astype(BF16)

    def step(size, rows, unit0, writes):
        plan, out, rolled, after = [], {}, {}, {}
        count = [0]
        true = lane >= -rows[2]
        even_ref = even_big_ref if size == BIG else even_small_ref

        def at(time, fn, *args):
            plan.append((time, len(plan), fn, args))

        def matmul(key, u, parts):
            lhs = _words(u_ref, (u,), 0, G)
            for reg, value in after.get(count[0], ()):
                keep = jnp.where(true, lhs[8 * reg:8 * reg + 8], value())
                lhs = jnp.concatenate(
                    ([lhs[:8 * reg]] if reg else []) + [keep, lhs[8 * reg + 8:]], axis=0)
            count[0] += 1
            res = jnp.dot(pltpu.bitcast(lhs, BF16), pltpu.bitcast(jnp.concatenate(parts, axis=0), BF16),
                          preferred_element_type=F32)
            for g in range(G):
                out[(*key, g)] = res[16 * g:16 * g + 16]

        def roll(t, odd, j):
            if ("e1", t, j) not in rolled:
                rolled["e1", t, j] = pltpu.roll(_words(d_ref, (t % 2, j, 1), 0, GD), 1, 1)
            if odd:
                rolled["e3", t, j] = pltpu.roll(_words(d_ref, (t % 2, j, 1), 0, GD), L - 1, 1)
            else:
                rolled["e0", t, j] = pltpu.roll(_words(d_ref, (t % 2, j, 0), 0, G), 2, 1)

        def multiply(t, odd, j):
            e1, e2 = rolled["e1", t, j], _words(d_ref, (t % 2, j, 0), 0, GD)
            if odd:
                matmul((t, odd, j, 0), 3 * j, [e2, rolled["e3", t, j]])
                matmul((t, odd, j, 1), 3 * j + 2,
                       [e1, _words(d_ref, (t % 2, j, 1), GD, 2), _words(d_ref, (t % 2, j, 2), 2, 2)])
            else:
                matmul((t, odd, j, 0), 3 * j, [e1, e2])
                matmul((t, odd, j, 1), 3 * j + 1,
                       [rolled["e0", t, j], _words(d_ref, (t % 2, j, 2), 0, 2)])

        def multiply_shared(t, i):
            def e2(r, g):
                if t >= EARLY:
                    return row_ref[staged(P, r, g)]
                lo = x0_ref[rows[r], pl.ds(8 * g, 8), :]
                hi = jnp.concatenate([x1_ref[rows[r], pl.ds(8 * g, 8), :], lo[:, W1:]], axis=1)
                return jnp.where(odd_lane, hi, lo)
            matmul((t, "s", i), 18, [e2(4 * t + i + a, g) for a in range(3) for g in range(GD, G)]
                   + [jnp.zeros((16, L), U32)])

        def acc(t, i, g):
            return t % 2, i, pl.ds(16 * g, 16), slice(None)

        def product(t, odd, j, g):
            return out.pop((t, odd, j, 0, g)) + out.pop((t, odd, j, 1, g))

        def emit(t, odd, i, g, y):
            ref = odd_ref if odd else even_ref
            ref[t % 2, i, pl.ds(16 * g, 16), :] = y.astype(BF16)
            if not odd:
                y_even = _words(even_ref, (t % 2, i), g, 1)
                y_odd = pltpu.roll(_words(odd_ref, (t % 2, i), g, 1), 1, 1)
                unit, reg = divmod((4 * t + i) * G + g, UNIT // 16)
                y0_ref[unit0 + unit, pl.ds(8 * reg, 8), :] = jnp.where(lo_from_odd, y_odd, y_even)
                y1_ref[unit0 + unit, pl.ds(8 * reg, 8), :] = jnp.where(lo_from_odd, y_even, y_odd)[:, :W1]

        def finish_shared(t, g):
            for i in range(4):
                acc_ref[acc(t, 8 + i, g)] = out.pop((t, "s", i, g))

        def finish_12(t, odd, g):
            a, b = product(t, odd, 1, g), product(t, odd, 2, g)
            s, d = a + b, a - b
            acc_ref[acc(t, 4 * odd, g)] = s
            acc_ref[acc(t, 4 * odd + 1, g)] = d

        def finish_34(t, odd, g):
            a, b = product(t, odd, 3, g), product(t, odd, 4, g)
            y = _output_transform(acc_ref[acc(t, 4 * odd, g)], acc_ref[acc(t, 4 * odd + 1, g)], a + b, a - b)
            s1, s2 = acc_ref[acc(t, 9, g)], acc_ref[acc(t, 10, g)]
            emit(t, odd, 1, g, y[1] + s1)
            emit(t, odd, 2, g, y[2] + s2)
            acc_ref[acc(t, 4 * odd + 2, g)] = y[0]
            acc_ref[acc(t, 4 * odd + 3, g)] = y[3]

        def finish_05(t, odd, g):
            first = product(t, odd, 0, g) + acc_ref[acc(t, 8, g)]
            last = product(t, odd, 5, g) + acc_ref[acc(t, 11, g)]
            y0, y3 = acc_ref[acc(t, 4 * odd + 2, g)], acc_ref[acc(t, 4 * odd + 3, g)]
            emit(t, odd, 0, g, y0 + first)
            emit(t, odd, 3, g, y3 + last)

        def transformed(slot, part, g, points):
            def value():
                v = _words(d_ref, (slot, points[0], part), g, 1)
                for j in points[1:]:
                    v = v | _words(d_ref, (slot, j, part), g, 1)
                return v
            return 0, value

        def emitted():
            unit, reg = divmod(G, UNIT // 16)
            idx = jnp.minimum(unit0 + unit, UNITS - 1), pl.ds(8 * reg, 8), slice(None)
            lo = y0_ref[idx]
            return jnp.concatenate([y1_ref[idx], lo[:, W1:]], axis=1)

        def shared_round(t, k):
            for i in range(4):
                at(k - 1, multiply_shared, t, i)
            for g in range(G):
                at(k + 1.35 + g / G, finish_shared, t, g)

        for t in range(EARLY):
            shared_round(t, t)
        k = EARLY
        for t in range(size):
            slot = (t + 1) % 2
            begin = k - 1.99 if t else -2
            for g in range(G):
                time = begin + 0.94 * g / G
                at(time, transform, slot, 4 * t + 4, g)
                for r in range(4 * t + (6 if t else 4), 4 * t + 10):
                    at(time - 0.42, interleave, rows, r, g)
                    if g >= GD:
                        at(time - 0.21, shift, r, g)
            pieces = ([(part, g) for g in range(GD) for part in range(2)]
                      + [(1, 4), (2, 2), None, (1, 5), (2, 3), None])
            due = k + len(ROUNDS) - (t < EARLY) + (EARLY <= t + 1 < size) + 2
            for q, piece in enumerate(pieces):
                if piece:
                    points = tuple(range(6)) if t + 1 == size else (1,)
                    index = int(4 * (due - 6.5 * (1 - q / len(pieces))))
                    assert index // 4 - 1 > begin + 1
                    after.setdefault(index, []).append(transformed(slot, *piece, points))

            for name in ROUNDS:
                if name == "s":
                    if t >= EARLY:
                        shared_round(t, k)
                        k += 1
                    continue
                odd = int(name[0] == "o")
                finish = {"12": finish_12, "34": finish_34, "05": finish_05}[name[1:]]
                for j in map(int, name[1:]):
                    at(k - 2.04, roll, t, odd, j)
                    at(k - 1, multiply, t, odd, j)
                for g in range(G):
                    at(k + 1.35 + g / G, finish, t, odd, g)
                k += 1
            after.setdefault(4 * (k + 3), []).insert(0, (1, emitted))
            for done, delay, starts in writes:
                if done == t + 1:
                    for q, start in enumerate(starts):
                        at(k + delay + 1.3 + q / 32, start)

        for _, _, fn, args in sorted(plan, key=lambda entry: entry[:2]):
            fn(*args)

    for copy in read_head():
        copy.wait()
    for g in range(G):
        for r in range(6):
            interleave([H - 2, H - 1, 0, 1, 2, 3], r, g)
    for g in range(GD, G):
        for r in range(6):
            shift(r, g)
    for g in range(G):
        transform(0, 0, g)

    def loop_body(size):
        def body(_, carry):
            s, base = carry
            rows = [base - 2 + r for r in range(4 * size + 6)]
            if size == SMALL:
                @pl.when(s < STEPS - 1)
                def _():
                    for copy in read(s, base + 4, 4 * size):
                        copy.wait()

                @pl.when(s == STEPS - 1)
                def _():
                    for copy in read_step(STEPS - 1):
                        copy.wait()

                rows[:2] = [jnp.where(r < 0, r + H, r) for r in rows[:2]]
                rows[-4:] = [jnp.where(r >= H, r - H, r) for r in rows[-4:]]
            else:
                for copy in read(s, base + 4, 4 * size):
                    copy.wait()
            writes = [(done, delay, [lambda start=start, on=on: pl.when(s == on)(start)
                                     for start in write_batch(n)])
                      for n, (on, done, delay) in enumerate(WRITES) if SIZES[on] == size]
            step(size, rows, (base >> 3) * (8 * C // UNIT), writes)
            return s + 1, base + 4 * size
        return body

    def segment(i, carry):
        for col, size in enumerate((SMALL, BIG)):
            trips = jnp.where(i == 0, SEGMENTS[0][col], SEGMENTS[1][col])
            carry = lax.fori_loop(0, trips, loop_body(size), carry)
        return carry

    lax.fori_loop(0, len(SEGMENTS), segment, (jnp.int32(0), jnp.int32(0)))

    for start in write_batch(len(WRITES)):
        start()
    for half in range(2):
        write(half, pl.ds(0, UNITS), pl.ds(0, UNIT)).wait()


@jax.jit
def pallas_standalone__fft_conv__vision_kernel(x: jax.Array, w: jax.Array):
    assert x.shape == (1, H, W, C) and w.shape == (3, 3, C, C)
    assert x.dtype == BF16 and w.dtype == BF16
    y = pl.pallas_call(
        _kernel,
        in_specs=[pl.BlockSpec(memory_space=pl.ANY), pl.BlockSpec(memory_space=pl.ANY)],
        out_specs=pl.BlockSpec(memory_space=pl.ANY),
        out_shape=jax.ShapeDtypeStruct((UNITS, UNIT, W), BF16),
        scratch_shapes=[
            pltpu.VMEM((H, C // 2, L), U32),
            pltpu.VMEM((H, C // 2, W1), U32),
            pltpu.VMEM((UNITS, UNIT // 2, L), U32),
            pltpu.VMEM((UNITS, UNIT // 2, W1), U32),
            pltpu.VMEM((3, 3, C, C), BF16),
            pltpu.VMEM((19, C, L), BF16),
            pltpu.VMEM((2, 6, 3, C, L), BF16),
            pltpu.VMEM((2, 4, C, L), BF16),
            pltpu.VMEM((2, 4, C, L), BF16),
            pltpu.VMEM((2, 4, C, L), BF16),
            pltpu.VMEM((4, RING, C // 2, L), U32),
            pltpu.VMEM((2, 12, C, L), F32),
            pltpu.SemaphoreType.DMA((STEPS + 1,)),
            pltpu.SemaphoreType.DMA(()),
            pltpu.SemaphoreType.DMA(()),
        ],
        compiler_params=pltpu.CompilerParams(
            vmem_limit_bytes=48 * 2**20, disable_semaphore_checks=True),
        name="fft_conv",
    )(jnp.transpose(x.reshape(H, W, C), (0, 2, 1)), w)
    return jnp.transpose(y.reshape(H, C, W), (0, 2, 1)).reshape(1, H, W, C)
```
